```python
import os as _os
_os.environ.setdefault('JAX_PLATFORMS', 'cpu')
import jax
import jax.numpy as jnp

def _softmax(x, axis=-1):
    return jax.nn.softmax(x, axis=axis)

def _gelu(x):
    return jax.nn.gelu(x, approximate=True)

def _silu(x):
    return jax.nn.silu(x)

def _sigmoid(x):
    return jax.nn.sigmoid(x)

def _layernorm(x, axis=-1, eps=1e-05):
    m = jnp.mean(x, axis=axis, keepdims=True)
    v = jnp.var(x, axis=axis, keepdims=True)
    return (x - m) / jnp.sqrt(v + eps)

def _scatter_add(tgt, idx, src, axis=0):
    return tgt.at[idx].add(src)

def _segment_sum(src, seg, n):
    return jax.ops.segment_sum(src, seg, n)

class _Rng:

    def __init__(self, key):
        self._k = key

    def _next(self):
        self._k, sub = jax.random.split(self._k)
        return sub

    def normal(self, shape):
        return jax.random.normal(self._next(), shape, dtype=jnp.bfloat16)

    def randint(self, lo, hi, shape):
        return jax.random.randint(self._next(), shape, lo, hi, dtype=jnp.int32)

    def uniform(self, shape, lo=0.0, hi=1.0):
        return jax.random.uniform(self._next(), shape, jnp.bfloat16, lo, hi)

    def permutation(self, n):
        return jax.random.permutation(self._next(), n)
kernel_name = 'concat_heads__linear_kernel_hedgehog__memory_aug_recurrent_mem_tr__prompt'

def setup_inputs():
    _rng = _Rng(jax.random.key(int.from_bytes(__import__("os").urandom(4), "little")))
    _w = lambda a: (lambda t: t.astype(jnp.bfloat16) if jnp.issubdtype(t.dtype, jnp.floating) else t)(jnp.asarray(a))

    def _A_setup():
        B, S, D, H = (1, 2048, 576, 32)
        Dh = D // H
        return {'x': _w((lambda *s: _rng.normal(s) * 0.4)(B, S, D)), 'wqkv': _w((lambda *s: _rng.normal(s) * 0.4)(D, 3 * D)), 'w_phi': _w((lambda *s: _rng.normal(s) * 0.4)(H, Dh, Dh) * Dh ** (-0.5)), 'wo': _w((lambda *s: _rng.normal(s) * 0.05)(D, D))}
    _A_in = _A_setup()

    def _B_setup():
        B, S, Dm = (1, 2048, 576)
        H, Dh = (32, 128)
        M, seg = (8, 32)
        seg = min(seg, S)
        S = S // seg * seg
        return {'x': _w((lambda *s: _rng.normal(s) * 0.05)(B, S, Dm)), 'mem0': _w((lambda *s: _rng.normal(s) * 0.8)(B, M, Dm)), 'Wq': _w((lambda *s: _rng.normal(s) * 3.2)(Dm, H, Dh) * Dm ** (-0.5)), 'Wk': _w((lambda *s: _rng.normal(s) * 3.2)(Dm, H, Dh) * Dm ** (-0.5)), 'Wv': _w((lambda *s: _rng.normal(s) * 0.8)(Dm, H, Dh) * Dm ** (-0.5)), 'Wo': _w((lambda *s: _rng.normal(s) * 0.8)(H, Dh, Dm) * (H * Dh) ** (-0.5)), 'seg_len': seg}
    _B_in = _B_setup()
    return {'A_x': _A_in['x'], 'A_wqkv': _A_in['wqkv'], 'A_w_phi': _A_in['w_phi'], 'A_wo': _A_in['wo'], 'B_x': _B_in['x'], 'B_mem0': _B_in['mem0'], 'B_Wq': _B_in['Wq'], 'B_Wk': _B_in['Wk'], 'B_Wv': _B_in['Wv'], 'B_Wo': _B_in['Wo'], 'B_seg_len': _B_in['seg_len']}

def reference(A_x, A_wqkv, A_w_phi, A_wo, B_x, B_mem0, B_Wq, B_Wk, B_Wv, B_Wo, B_seg_len):

    def _A_ref(x, wqkv, w_phi, wo):
        B, S, D = x.shape
        H = 32
        Dh = D // H
        qkv = (lambda x, *d: x.transpose(*d))((x @ wqkv).reshape(B, S, 3, H, Dh), 2, 0, 3, 1, 4)
        q, k, v = (qkv[0], qkv[1], qkv[2])
        pq = jnp.einsum('bhsd,hdf->bhsf', q, w_phi)
        pk = jnp.einsum('bhsd,hdf->bhsf', k, w_phi)
        phi_q = jnp.concatenate([_softmax(pq, axis=-1), _softmax(-pq, axis=-1)], axis=-1)
        phi_k = jnp.concatenate([_softmax(pk, axis=-1), _softmax(-pk, axis=-1)], axis=-1)
        kv = jnp.einsum('bhsf,bhsd->bhfd', phi_k, v)
        z = jnp.einsum('bhsf->bhf', phi_k)
        num = jnp.einsum('bhqf,bhfd->bhqd', phi_q, kv)
        den = jnp.einsum('bhqf,bhf->bhq', phi_q, z)[..., None] + 1e-06
        o = num / den
        return (lambda x, *d: x.transpose(*d))(o, 0, 2, 1, 3).reshape(B, S, D) @ wo

    def _B_ref(x, mem0, Wq, Wk, Wv, Wo, seg_len):
        B, S, Dm = x.shape
        H, Dh = (Wq.shape[1], Wq.shape[2])
        M = mem0.shape[1]
        scale = Dh ** (-0.5)
        n_seg = S // seg_len
        L = M + seg_len
        idx = jnp.arange(L)
        mask = (idx[:, None] < M) | (idx[:, None] >= idx[None, :])
        mem = mem0
        outs = []
        for s in range(n_seg):
            xs = x[:, s * seg_len:(s + 1) * seg_len, :].copy()
            h = jnp.concatenate([mem, xs], axis=1)
            q = jnp.einsum('btd,dhe->bhte', h, Wq)
            k = jnp.einsum('btd,dhe->bhte', h, Wk)
            v = jnp.einsum('btd,dhe->bhte', h, Wv)
            scores = jnp.einsum('bhqe,bhke->bhqk', q, k) * scale
            scores = jnp.where(mask[None, None], scores, -1000000000.0)
            p = _softmax(scores, axis=-1)
            o = jnp.einsum('bhqk,bhke->bhqe', p, v)
            o = jnp.einsum('bhte,hed->btd', o, Wo)
            mem = o[:, :M, :].copy()
            outs.append(o[:, M:, :])
        return jnp.concatenate(outs, axis=1)
    a = _A_ref(A_x, A_wqkv, A_w_phi, A_wo)
    b = _B_ref(B_x, B_mem0, B_Wq, B_Wk, B_Wv, B_Wo, B_seg_len)
    return jnp.concatenate([a, b], axis=-1)
```

```python
import functools

import jax
import jax.numpy as jnp
from jax import lax
import jax.experimental.pallas as pl
import jax.experimental.pallas.tpu as pltpu

F32 = jnp.float32
BF16 = jnp.bfloat16
U32 = jnp.uint32
I32 = jnp.int32
NT = (((1,), (1,)), ((), ()))
TN = (((0,), (0,)), ((), ()))
LOG2E = 1.4426950408889634

S = 2048
D = 576
HA = 32
DA = 18
GA = 8
NG = HA // GA
RG = DA * GA
HR = RG // 2
HB = 32
DB = 128
MEM = 8
SEG = 32
TB = 128
NSTEP = S // TB
CH = 6
NPIECE = 3 * (D // 16) // CH
PROWS = CH * 16 * HB
NWO = 8
NXA = 4
LAGS = (2, 4, 6)
RLAST = 1
SEM_WQKV, SEM_WOA, SEM_XA = 0, 1, 2
SEM_RAW = SEM_XA + NXA
SEM_WO = SEM_RAW + NPIECE
NSEM = SEM_WO + NWO


def _iota(shape, dim):
    return lax.broadcasted_iota(I32, shape, dim)


def _recip(x):
    r = pl.reciprocal(x, approx=True)
    return r * (2.0 - x * r)


def _b16(v):
    return pltpu.bitcast(v, BF16)


def _u32(v):
    return pltpu.bitcast(v, U32)


def _dot(a, b):
    return jnp.dot(a, b, preferred_element_type=F32)


def _dot_nt(a, b):
    return lax.dot_general(a, b, NT, preferred_element_type=F32)


def _feature_map(pk):
    t = pk.shape[-1]
    x = pk.reshape(DA, GA, t)
    mx = jnp.max(x, axis=0, keepdims=True)
    mn = jnp.min(x, axis=0, keepdims=True)
    ep = jnp.exp2(x - mx)
    en = jnp.exp2(mn - x)
    rp = _recip(jnp.sum(ep, axis=0, keepdims=True))
    rn = _recip(jnp.sum(en, axis=0, keepdims=True))
    pp = (ep * rp).reshape(RG, t).astype(BF16)
    pn = (en * rn).reshape(RG, t).astype(BF16)
    return jnp.concatenate([pp, pn], axis=0)


def _kernel(xat_hbm, wqkv_hbm, wphi_ref, woa_hbm, xbt_ref, xbn_ref, mem0_ref, wq_hbm, wk_hbm, wv_hbm, wobt_hbm,
            o_ref,
            xat, wqkv, woa, raw, stage, wr, wobt, wob, wt, wop, kvacc, kvl,
            mem, sq, sk, sv, biasa, biasb, pqs, xbs, sems, *, do_a, do_b):
    step = pl.program_id(0)
    scale = DB ** (-0.5)

    @pl.when(step == 0)
    def _prologue():
        XW = S // NXA
        c_wqkv = pltpu.make_async_copy(wqkv_hbm, wqkv, sems.at[SEM_WQKV])
        c_woa = pltpu.make_async_copy(woa_hbm, woa, sems.at[SEM_WOA])
        c_xa = [pltpu.make_async_copy(xat_hbm.at[:, pl.ds(i * XW, XW)], xat.at[:, pl.ds(i * XW, XW)],
                                      sems.at[SEM_XA + i]) for i in range(NXA)]
        c_wqkv.start()
        c_woa.start()
        for c in c_xa:
            c.start()
        ppm = NPIECE // 3
        for p in range(NPIECE):
            src = (wq_hbm, wk_hbm, wv_hbm)[p // ppm]
            pltpu.make_async_copy(src.at[pl.ds((p % ppm) * PROWS, PROWS)], raw.at[pl.ds(p * PROWS, PROWS)],
                                  sems.at[SEM_RAW + p]).start()
        hpw = HB // NWO
        for p in range(NWO):
            pltpu.make_async_copy(wobt_hbm.at[pl.ds(p * hpw, hpw)], wobt.at[pl.ds(p * hpw, hpw)],
                                  sems.at[SEM_WO + p]).start()

        neg = -1e9 / scale
        r = _iota((32, 48), 0)
        c = _iota((32, 48), 1)
        valid = (c < 40) & ((r < 8) | (r >= c))
        biasa[...] = jnp.where(valid, 0.0, jnp.where(c < 40, neg, -jnp.inf)).astype(F32)
        r = _iota((48, 80), 0)
        c = _iota((48, 80), 1)
        q_is_a = (r >= 32) & (r < 40)
        qi = jnp.where(r < 8, r, jnp.where(r < 32, r + 8, jnp.where(r < 40, r, r - 32)))
        k_is_a = c < 40
        kj = jnp.where(c < 40, c, jnp.where(c < 48, c - 32, jnp.where(c < 56, c - 48, c - 40)))
        same = q_is_a == k_is_a
        valid = same & ((qi < 8) | (qi >= kj))
        biasb[...] = jnp.where(valid, 0.0, jnp.where(same, neg, -jnp.inf)).astype(F32)
        mem[...] = mem0_ref[...].astype(F32)
        kvacc[...] = jnp.zeros(kvacc.shape, F32)

        W = 256
        hl = _iota((GA, W), 0)

        def split(off, rows):
            cc = _iota((rows, W), 1) - off
            hh = jnp.floor((cc.astype(F32) + 0.5) * (1.0 / DA)).astype(I32)
            return hh, cc - hh * DA

        def selectors(g, off):
            h32, d32 = split(off, HA)
            hsel = h32 == _iota((HA, W), 0) - g * GA
            hsel = hsel & (h32 >= 0) & (h32 < GA)
            t1 = jnp.zeros((DA, W), F32)
            for d in range(DA):
                sp = jnp.where(hsel & (d32 == d), 1.0, 0.0).astype(BF16)
                t1 = t1 + _dot(wphi_ref[d], sp)
            h_c, d_c = split(off, GA)
            hm = h_c == hl
            bd = [jnp.where(hm, jnp.broadcast_to(t1[f:f + 1, :], (GA, W)), 0.0) for f in range(DA)]
            pm = [jnp.where(hm & (d_c == f), 1.0, 0.0) for f in range(DA)]
            return (jnp.concatenate(bd, axis=0).astype(BF16), jnp.concatenate(pm, axis=0).astype(BF16))

        sel_q = [selectors(g, 16 * g) for g in range(NG)]
        sel_k = [selectors(g, 64 + 16 * g)[0] for g in range(NG)]
        c_wqkv.wait()
        for g in range(NG):
            rows = slice(g * HR, (g + 1) * HR)
            wk_ = min(W, 3 * D - (1152 + 128 * g))
            wt[1, rows, :] = _u32((_dot_nt(sel_k[g], wqkv[:, 512 + 128 * g:512 + 128 * g + W]) * LOG2E).astype(BF16))
            wt[2, rows, :] = _u32(_dot_nt(sel_q[g][1][:, :wk_],
                                          wqkv[:, 1152 + 128 * g:1152 + 128 * g + wk_]).astype(BF16))
        for g in range(NG):
            rows = slice(g * HR, (g + 1) * HR)
            wt[0, rows, :] = _u32((_dot_nt(sel_q[g][0], wqkv[:, 128 * g:128 * g + W]) * LOG2E).astype(BF16))
        c_woa.wait()
        wps = []
        for g in range(NG):
            wk_ = min(W, D - 128 * g)
            wps.append(_dot(sel_q[g][1][:, :wk_], woa[128 * g:128 * g + wk_, :]).astype(BF16))
        wop[...] = _u32(jnp.concatenate(wps, axis=0).astype(F32).T.astype(BF16))

        ones = jnp.ones((16, TB), BF16)

        def phase1(i, extra=()):
            extra = list(extra)
            xv = xat.at[:, pl.ds(pl.multiple_of(i * TB, TB), TB)]
            pks, vts, phis = {}, {}, {}

            def more(n, last=False):
                if RLAST and not last:
                    return
                for _ in range(n):
                    if extra:
                        extra.pop(0)()
            for t in range(NG + 2):
                if t < NG:
                    pks[t] = _dot(_b16(wt[1, t * HR:(t + 1) * HR, :]), xv[...])
                    more(1)
                    vt = _dot(_b16(wt[2, t * HR:(t + 1) * HR, :]), xv[...])
                    more(1)
                    vts[t] = jnp.concatenate([vt.astype(BF16), ones], axis=0)
                    phis[t] = _feature_map(pks.pop(t))
                g = t - 2
                if g >= 0:
                    kvacc[g] += _dot_nt(vts.pop(g), phis.pop(g))
                    more(1)
            more(len(extra), True)

        def relayout_parts(p):
            r0 = pl.multiple_of(p * PROWS, PROWS)
            rawp = raw.at[pl.ds(r0, PROWS)]
            pltpu.make_async_copy(rawp, rawp, sems.at[SEM_RAW + p]).wait()
            m = p // (NPIECE // 3)
            d0 = (p - m * (NPIECE // 3)) * (CH * 8)
            parts = []
            for c in range(CH):
                def put(c=c):
                    st = stage.at[c % 2]
                    for q in range(8):
                        v = rawp[c * 512 + q * 64:c * 512 + (q + 1) * 64, :]
                        st[pl.ds(q * 33, 32), :] = _u32(v)

                def get(c=c):
                    st = stage.at[c % 2]
                    rr = pl.multiple_of(d0 + c * 8, 8)
                    for j in range(16):
                        e = st[pl.ds(j, 8, stride=33), :]
                        o = st[pl.ds(16 + j, 8, stride=33), :]
                        wr[(2 * j) * 3 + m, pl.ds(rr, 8), :] = (e & U32(0xffff)) | (o << 16)
                        wr[(2 * j + 1) * 3 + m, pl.ds(rr, 8), :] = (e >> 16) | (o & U32(0xffff0000))
                parts += [put, get]
            return parts

        def relayout(p):
            for f in relayout_parts(p):
                f()

        SH = 2
        c_xa[0].wait()

        def l1(i, carry):
            if do_a:
                phase1(i)
            return carry
        lax.fori_loop(0, SH, l1, 0)
        for c in c_xa[1:]:
            c.wait()

        def l2(i, carry):
            if do_a:
                phase1(i, relayout_parts(i - SH))
            else:
                relayout(i - SH)
            return carry
        lax.fori_loop(SH, NSTEP, l2, 0)

        r = _iota((RG + 16, 2 * RG), 0)
        c = _iota((RG + 16, 2 * RG), 1)
        keep = ((r & (GA - 1)) == (c & (GA - 1))) & (r < RG + GA)
        for g in range(NG):
            kvl[g] = _u32(jnp.where(keep, kvacc[g], 0.0).astype(BF16))

        xbs[...] = xbt_ref[...].astype(F32).T
        for g in range(NG):
            pqs[g * RG:(g + 1) * RG, :] = _dot(_b16(wt[0, g * HR:(g + 1) * HR, :]), xat[:, 0:TB])

        def l3(p, carry):
            relayout(p)
            return carry
        lax.fori_loop(NSTEP - SH, NPIECE, l3, 0)

        def tr(p, carry):
            h0 = pl.multiple_of(p * hpw, hpw)
            pltpu.make_async_copy(wobt.at[pl.ds(h0, hpw)], wobt.at[pl.ds(h0, hpw)], sems.at[SEM_WO + p]).wait()
            for hh in range(hpw):
                h = h0 + hh
                r0 = pl.multiple_of(h * 64, 64)
                for j in range(4):
                    blk = wobt[h, j * 128:(j + 1) * 128, :].astype(F32)
                    wob[j, pl.ds(r0, 64), :] = _u32(blk.T.astype(BF16))
                blk = jnp.concatenate([wobt[h, 512:576, :].astype(F32), jnp.zeros((64, DB), F32)], axis=0)
                wob[4, pl.ds(r0, 64), :] = _u32(blk.T.astype(BF16))
            return carry
        lax.fori_loop(0, NWO, tr, 0)

    st2 = {}

    def a_pq(g):
        def f():
            if "x" not in st2:
                nxt = jnp.minimum(step + 1, NSTEP - 1)
                st2["x"] = xat.at[:, pl.ds(pl.multiple_of(nxt * TB, TB), TB)]
            pqs[g * RG:(g + 1) * RG, :] = _dot(_b16(wt[0, g * HR:(g + 1) * HR, :]), st2["x"][...])
        return f

    def a_phi(g):
        def f():
            st2["phi", g] = _feature_map(pqs[g * RG:(g + 1) * RG, :])
        return f

    def b_xt():
        xbs[...] = xbn_ref[...].astype(F32).T

    def a_num(g):
        def f():
            r = _dot(_b16(kvl[g]), st2.pop(("phi", g)))
            den = r[RG:RG + GA, :] + 1e-6
            o = r[:RG, :].reshape(DA, GA, TB) * (1.0 / den)[None]
            st2["o", g] = o.reshape(RG, TB).astype(BF16)
        return f

    def a_out(g):
        def f():
            if "ot" not in st2:
                st2["ot"] = jnp.concatenate([st2.pop(("o", k)) for k in range(NG)], axis=0)
            st2["out", g] = _dot(_b16(wop[g * HR:(g + 1) * HR, :]), st2["ot"])
            if g == NG - 1:
                outa = jnp.concatenate([st2.pop(("out", k)) for k in range(NG)], axis=0).T
                o_ref[:, 0:D] = outa.astype(BF16)
        return f

    E = HB + LAGS[2] - 1
    pq, phi, num, out, xt = a_pq, a_phi, a_num, a_out, b_xt
    fills = [{4: [phi(0)], 10: [phi(1)], 16: [phi(2)], 22: [phi(3)],
              E - 4: [num(0)], E - 2: [num(1)], E: [num(2), num(3)]},
             {E - 4: [out(0)], E - 2: [out(1)], E: [out(2)]},
             {4: [xt], E - 2: [out(3)], E: [pq(0)]},
             {E - 4: [pq(1)], E - 2: [pq(2)], E: [pq(3)]}]
    if not do_a:
        fills = [{}, {}, {}, {20: [b_xt]}]
        o_ref[:, 0:D] = jnp.zeros((TB, D), BF16)

    cexp = scale * LOG2E

    def b_step(hmat, first, fill):
        bias = biasa[...] if first else biasb[...]
        ok = bias == 0.0
        acc = None
        qkv = {}
        pv = {}
        oo = {}

        def proj(h):
            q, k, v = [_dot(hmat, _b16(wr[h * 3 + i])).astype(BF16) for i in range(3)]
            if first:
                sq[h] = _u32(q[32:48])
                sk[h] = _u32(k)
                sv[h] = _u32(v)
                q = q[0:32]
            else:
                q = jnp.concatenate([q, _b16(sq[h])], axis=0)
                k = jnp.concatenate([_b16(sk[h]), k], axis=0)
                v = jnp.concatenate([_b16(sv[h]), v], axis=0)
            qkv[h] = (q, k, v)

        def score(h):
            q, k, v = qkv.pop(h)
            s = _dot_nt(q, k)
            s = jnp.where(ok, s, bias)
            m = jnp.max(s, axis=-1, keepdims=True)
            p = jnp.exp2((s - m) * cexp)
            l = jnp.sum(p, axis=-1, keepdims=True)
            pv[h] = (p.astype(BF16), l, v)

        def mix(h):
            p, l, v = pv.pop(h)
            oo[h] = (_dot(p, v) * _recip(l)).astype(BF16)

        def outp(h, acc):
            o = oo.pop(h)
            parts = [_dot(o, _b16(wob[j, h * 64:(h + 1) * 64, :])) for j in range(5)]
            if acc is None:
                return parts
            return [a + b for a, b in zip(acc, parts)]

        la, lb, lc = LAGS
        for t in range(HB + lc):
            if t < HB:
                proj(t)
            if 0 <= t - la < HB:
                score(t - la)
            if 0 <= t - lb < HB:
                mix(t - lb)
            if 0 <= t - lc < HB:
                acc = outp(t - lc, acc)
            for f in fill.get(t, ()):
                f()
        acc[4] = acc[4][:, 0:64]
        return jnp.concatenate(acc, axis=1)

    if do_b:
        m_cur = mem[...]
        xs = [xbs[p * 64:(p + 1) * 64, :] for p in range(2)]
        for p in range(TB // (2 * SEG)):
            x = xs[p]
            ha = jnp.concatenate([m_cur, x[0:40]], axis=0).astype(BF16)
            ra = b_step(ha, True, fills[2 * p])
            hb = jnp.concatenate([ra[0:8], x[40:64]], axis=0).astype(BF16)
            rb = b_step(hb, False, fills[2 * p + 1])
            m_cur = rb[0:8]
            ob = jnp.concatenate([ra[8:32], rb[32:48], rb[8:32]], axis=0)
            o_ref[p * 64:(p + 1) * 64, D:2 * D] = ob.astype(BF16)
        mem[...] = m_cur
    else:
        for fl in fills:
            for t in sorted(fl):
                for f in fl[t]:
                    f()
        o_ref[:, D:2 * D] = jnp.zeros((TB, D), BF16)


@functools.partial(jax.jit, static_argnames=("B_seg_len", "do_a", "do_b", "nsteps"))
def pallas_concat_heads__linear_kernel_hedgehog__memory_aug_recurrent_mem_tr__prompt_kernel(A_x, A_wqkv, A_w_phi, A_wo, B_x, B_mem0, B_Wq, B_Wk, B_Wv, B_Wo, B_seg_len,
           do_a=True, do_b=True, nsteps=NSTEP):
    assert B_seg_len == SEG
    hbm = pl.BlockSpec(memory_space=pltpu.HBM)
    out = pl.pallas_call(
        functools.partial(_kernel, do_a=do_a, do_b=do_b),
        grid=(nsteps,),
        in_specs=[
            hbm, hbm,
            pl.BlockSpec((DA, DA, HA), lambda i: (0, 0, 0)),
            hbm,
            pl.BlockSpec((D, TB), lambda i: (0, 0)),
            pl.BlockSpec((D, TB), lambda i: (0, jnp.minimum(i + 1, NSTEP - 1))),
            pl.BlockSpec((MEM, D), lambda i: (0, 0)),
            hbm, hbm, hbm, hbm,
        ],
        out_specs=pl.BlockSpec((TB, 2 * D), lambda i: (i, 0)),
        out_shape=jax.ShapeDtypeStruct((S, 2 * D), BF16),
        scratch_shapes=[
            pltpu.VMEM((D, S), BF16),
            pltpu.VMEM((D, 3 * D), BF16),
            pltpu.VMEM((D, D), BF16),
            pltpu.VMEM((3 * D * HB, DB), BF16),
            pltpu.VMEM((2, 8 * 33, 128), U32),
            pltpu.VMEM((3 * HB, D // 2, DB), U32),
            pltpu.VMEM((HB, D, DB), BF16),
            pltpu.VMEM((5, HB * DB // 2, 128), U32),
            pltpu.VMEM((3, D // 2, D), U32),
            pltpu.VMEM((D // 2, D), U32),
            pltpu.VMEM((NG, RG + 16, 2 * RG), F32),
            pltpu.VMEM((NG, (RG + 16) // 2, 2 * RG), U32),
            pltpu.VMEM((MEM, D), F32),
            pltpu.VMEM((HB, 8, DB), U32),
            pltpu.VMEM((HB, 24, DB), U32),
            pltpu.VMEM((HB, 24, DB), U32),
            pltpu.VMEM((32, 48), F32),
            pltpu.VMEM((48, 80), F32),
            pltpu.VMEM((D, TB), F32),
            pltpu.VMEM((TB, D), F32),
            pltpu.SemaphoreType.DMA((NSEM,)),
        ],
        compiler_params=pltpu.CompilerParams(
            dimension_semantics=("arbitrary",),
            vmem_limit_bytes=100 * 1024 * 1024,
        ),
        name="hedgehog_memtr",
    )(
        A_x[0].T, A_wqkv, jnp.transpose(A_w_phi, (1, 2, 0)), A_wo,
        B_x[0].T, B_x[0].T, B_mem0.reshape(MEM, D),
        B_Wq.reshape(D * HB, DB), B_Wk.reshape(D * HB, DB), B_Wv.reshape(D * HB, DB),
        jnp.transpose(B_Wo, (0, 2, 1)),
    )
    return out.reshape(1, S, 2 * D)
```

```python
import functools

import jax
import jax.numpy as jnp
from jax import lax
import jax.experimental.pallas as pl
import jax.experimental.pallas.tpu as pltpu

F32 = jnp.float32
BF16 = jnp.bfloat16
U32 = jnp.uint32
I32 = jnp.int32
NT = (((1,), (1,)), ((), ()))
LOG2E = 1.4426950408889634

S = 2048
D = 576
HA = 32
DA = 18
NP = 4
HP = 72
RG = 72
NG = 8
HB = 32
DB = 128
MEM = 8
SEG = 32
TB = 128
NSTEP = S // TB
T1 = 256
CH = 18
NPIECE = 3 * (D // 16) // CH
PROWS = CH * 16 * HB
HW = 3
WO_PIECES = [(p * HW, HW) for p in range(NPIECE)] + [(18, 7), (25, 7)]
NWO = len(WO_PIECES)
PACE = 4
SPN = 10
LAG_SCORE, LAG_MIX, LAG_OUT = 2, 5, 7
OUT_RATE = 3
NO = 3
(SEM_WK, SEM_WV, SEM_WQ, SEM_WOA, SEM_XA0, SEM_XA1, SEM_PHI, SEM_MEM, SEM_XB0, SEM_XB1, SEM_WO) = range(11)
SEM_RAW = SEM_WO + NWO
NSEM = SEM_RAW + NPIECE


def _iota(shape, dim):
    return lax.broadcasted_iota(I32, shape, dim)


def _recip(x):
    r = pl.reciprocal(x, approx=True)
    return r * (2.0 - x * r)


def _b16(v):
    return pltpu.bitcast(v, BF16)


def _u32(v):
    return pltpu.bitcast(v, U32)


def _dot(a, b):
    return jnp.dot(a, b, preferred_element_type=F32)


def _dot_nt(a, b):
    return lax.dot_general(a, b, NT, preferred_element_type=F32)


def _feature_map(p):
    t = p.shape[-1]
    x = p.reshape(DA // 2, 8, t)

    def both(r, op):
        return op(r, pltpu.roll(r, 4, 0))[None]
    mx = both(jnp.max(x, axis=0), jnp.maximum)
    mn = both(jnp.min(x, axis=0), jnp.minimum)
    ep = jnp.exp2(x - mx)
    en = jnp.exp2(mn - x)
    rp = _recip(both(jnp.sum(ep, axis=0), jnp.add))
    rn = _recip(both(jnp.sum(en, axis=0), jnp.add))
    return jnp.concatenate([ep * rp, en * rn], axis=0).reshape(2 * RG, t).astype(BF16)


def _pace(res, n):
    pos = [(r, c) for c in range(res.shape[1] // 128) for r in range(res.shape[0] // 8)]
    pos = [pos[(2 * i + 1) * len(pos) // (2 * n)] for i in range(n)]
    return [(_u32(res[8 * r:8 * r + 8, 128 * c:128 * c + 128]) >> 16) >> 16 for r, c in pos]


def _spread(fs, n, total):
    return [fs[len(fs) * k // n:len(fs) * (k + 1) // n] for k in range(n)] + [[]] * (total - n)


def _kernel(xat_hbm, wqkv_hbm, wphi_hbm, woa_hbm, xbt_hbm, mem0_hbm, wq_hbm, wk_hbm, wv_hbm, wobt_hbm,
            o_ref,
            xat, wqkv, woa, raw, stage, wr, wobt, wob, wt, wop, kvacc, kvl, phq,
            mem, sq, sk, sv, biasa, biasb, xbs, wphi, mem0, xbt, nums, sems):
    step = pl.program_id(0)
    scale = DB ** (-0.5)

    def cols(src, dst, a, b, sem):
        return pltpu.make_async_copy(src.at[:, pl.ds(a, b - a)], dst.at[:, pl.ds(a, b - a)], sems.at[sem])

    @pl.when(step == 0)
    def _prologue():
        c_phi = pltpu.make_async_copy(wphi_hbm, wphi, sems.at[SEM_PHI])
        c_wk = cols(wqkv_hbm, wqkv, 512, 1152, SEM_WK)
        c_wv = cols(wqkv_hbm, wqkv, 1152, 1728, SEM_WV)
        c_wq = cols(wqkv_hbm, wqkv, 0, 512, SEM_WQ)
        c_xa0 = cols(xat_hbm, xat, 0, 2 * T1, SEM_XA0)
        c_xa1 = cols(xat_hbm, xat, 2 * T1, S, SEM_XA1)
        c_woa = pltpu.make_async_copy(woa_hbm, woa, sems.at[SEM_WOA])
        c_mem = pltpu.make_async_copy(mem0_hbm, mem0, sems.at[SEM_MEM])
        c_xb0 = cols(xbt_hbm, xbt, 0, 2 * TB, SEM_XB0)
        for c in (c_phi, c_wk, c_wv, c_wq, c_xa0, c_xa1):
            c.start()
        for p in range(NWO):
            if p < NPIECE:
                src = (wq_hbm, wk_hbm, wv_hbm)[p // 2]
                pltpu.make_async_copy(src.at[pl.ds((p % 2) * PROWS, PROWS)], raw.at[pl.ds(p * PROWS, PROWS)],
                                      sems.at[SEM_RAW + p]).start()
            if p == NPIECE:
                for c in (c_woa, c_mem, c_xb0):
                    c.start()
            pltpu.make_async_copy(wobt_hbm.at[pl.ds(*WO_PIECES[p])], wobt.at[pl.ds(*WO_PIECES[p])],
                                  sems.at[SEM_WO + p]).start()
        cols(xbt_hbm, xbt, 2 * TB, S, SEM_XB1).start()
        c_phi.wait()

        W = 256
        WF = 640

        def split(off, shape):
            cc = _iota(shape, 1) - off
            hh = jnp.floor((cc.astype(F32) + 0.5) * (1.0 / DA)).astype(I32)
            return hh, cc - hh * DA

        wcat = jnp.concatenate([wphi[d].astype(F32) for d in range(DA)], axis=1).astype(BF16)
        rr = _iota((D, WF), 0)
        t1s = []
        for off in (0, 64):
            hh, dd = split(off, (8, WF))
            src = jnp.where((hh >= 0) & (hh < HA), dd * HA + hh, -1)[0:1, :]
            t1s.append(_dot(wcat, jnp.where(rr == src, 1.0, 0.0).astype(BF16)))
        sub = _iota((8, W), 0)
        lo = sub < 4

        def selectors(p, k):
            h_c, d_c = split(16 * p + 64 * k, (8, W))
            t1 = t1s[k][:, 128 * p:128 * p + W]
            bd, pm = [], []
            for g2 in range(2):
                hm = h_c == (sub & 3) + 4 * g2
                for fp in range(DA // 2):
                    row = jnp.where(lo, jnp.broadcast_to(t1[2 * fp:2 * fp + 1, :], (8, W)),
                                    jnp.broadcast_to(t1[2 * fp + 1:2 * fp + 2, :], (8, W)))
                    bd.append(jnp.where(hm, row, 0.0))
                    pm.append(jnp.where(hm & (d_c == 2 * fp + (sub >> 2)), 1.0, 0.0))
            return (jnp.concatenate(bd, axis=0).astype(BF16), jnp.concatenate(pm, axis=0).astype(BF16))

        sel_k = [selectors(p, 1)[0] for p in range(NP)]
        sel_q = [selectors(p, 0) for p in range(NP)]
        c_wk.wait()
        for p in range(NP):
            wt[1, p * HP:(p + 1) * HP, :] = _u32(
                (_dot_nt(sel_k[p], wqkv[:, 512 + 128 * p:512 + 128 * p + W]) * LOG2E).astype(BF16))
        c_wv.wait()
        c_wq.wait()
        c_xa0.wait()
        for j in range(5):
            n = 128 if j < 4 else 64
            blk = wqkv[:, 1152 + 128 * j:1152 + 128 * j + n].astype(F32)
            wt[2, 64 * j:64 * j + n // 2, :] = _u32(blk.T.astype(BF16))
        for p in range(NP):
            wt[0, p * HP:(p + 1) * HP, :] = _u32(
                (_dot_nt(sel_q[p][0], wqkv[:, 128 * p:128 * p + W]) * LOG2E).astype(BF16))

        neg = -1e9 / scale
        r = _iota((32, 48), 0)
        c = _iota((32, 48), 1)
        valid = (c < 40) & ((r < 8) | (r >= c))
        biasa[...] = jnp.where(valid, 0.0, jnp.where(c < 40, neg, -jnp.inf)).astype(F32)
        r = _iota((48, 80), 0)
        c = _iota((48, 80), 1)
        q_is_a = (r >= 32) & (r < 40)
        qi = jnp.where(r < 8, r, jnp.where(r < 32, r + 8, jnp.where(r < 40, r, r - 32)))
        k_is_a = c < 40
        kj = jnp.where(c < 40, c, jnp.where(c < 48, c - 32, jnp.where(c < 56, c - 48, c - 40)))
        same = q_is_a == k_is_a
        valid = same & ((qi < 8) | (qi >= kj))
        biasb[...] = jnp.where(valid, 0.0, jnp.where(same, neg, -jnp.inf)).astype(F32)
        kvacc[...] = jnp.zeros(kvacc.shape, F32)

        def phase1(i, extra=()):
            t0 = pl.multiple_of(i * T1, T1)
            xv = xat.at[:, pl.ds(t0, T1)]
            ones = jnp.ones((8, T1), F32)
            vts, phis = {}, {}

            def proj(m, t, k):
                res = _dot(_b16(wt[m, t * HP:(t + 1) * HP, :]), xv[...])
                if extra:
                    for f, z in zip(extra[k], _pace(res, len(extra[k]))):
                        f(z)
                return res
            for t in range(NP + 1):
                if t < NP:
                    pq = proj(0, t, 3 * t)
                    for g2 in range(2):
                        phq[2 * t + g2, :, pl.ds(t0, T1)] = _u32(_feature_map(pq[g2 * RG:(g2 + 1) * RG]))
                    pk = proj(1, t, 3 * t + 1)
                    vt = proj(2, t, 3 * t + 2)
                    for g2 in range(2):
                        vts[2 * t + g2] = jnp.concatenate([vt[g2 * RG:(g2 + 1) * RG], ones], axis=0).astype(BF16)
                        phis[2 * t + g2] = _feature_map(pk[g2 * RG:(g2 + 1) * RG])
                if t >= 1:
                    for g in (2 * t - 2, 2 * t - 1):
                        kvacc[g] += _dot_nt(vts.pop(g), phis.pop(g))

        def relayout(p):
            rawp = raw.at[pl.ds(pl.multiple_of(p * PROWS, PROWS), PROWS)]
            pltpu.make_async_copy(rawp, rawp, sems.at[SEM_RAW + p]).wait()
            m = p // 2
            d0 = (p - m * 2) * (CH * 8)

            def put(c, q0, z):
                st = stage.at[c % 2]
                for q in range(q0, q0 + 8 // PACE):
                    u = _u32(rawp[c * 512 + q * 64:c * 512 + (q + 1) * 64, :])
                    st[pl.ds(q * 33, 32), :] = u | jnp.concatenate([z] * 4, axis=0)

            def get(c, j0, z):
                st = stage.at[c % 2]
                rr = pl.multiple_of(d0 + c * 8, 8)
                for j in range(j0, j0 + 16 // PACE):
                    e = st[pl.ds(j, 8, stride=33), :] | z
                    o = st[pl.ds(16 + j, 8, stride=33), :]
                    wr[(2 * j) * 3 + m, pl.ds(rr, 8), :] = (e & U32(0xffff)) | (o << 16)
                    wr[(2 * j + 1) * 3 + m, pl.ds(rr, 8), :] = (e >> 16) | (o & U32(0xffff0000))
            fs = []
            for c in range(CH):
                fs += [functools.partial(put, c, k * 8 // PACE) for k in range(PACE)]
                fs += [functools.partial(get, c, k * 16 // PACE) for k in range(PACE)]
            return fs

        def transpose_wo(p):
            h0, hw = WO_PIECES[p] if isinstance(p, int) else (p * HW, HW)
            src = wobt.at[pl.ds(h0, hw)]
            pltpu.make_async_copy(src, src, sems.at[SEM_WO + p]).wait()
            dst = wob.at[:, pl.ds(pl.multiple_of(h0 * 64, 64), hw * 64), :]

            def block(hh, j, z):
                n = 128 if j < 4 else 64
                u = _u32(src[hh, j * 128:j * 128 + n, :])
                u = jnp.concatenate([u[0:8] | z, u[8:]] + ([] if j < 4 else [jnp.zeros((32, DB), U32)]), axis=0)
                dst[j, hh * 64:(hh + 1) * 64, :] = _u32(_b16(u).astype(F32).T.astype(BF16))
            return [functools.partial(block, hh, j) for hh in range(hw) for j in range(5)]

        def weave(a, b):
            out = []
            for k in range(len(b)):
                out += a[len(a) * k // len(b):len(a) * (k + 1) // len(b)] + [b[k]]
            return out

        def l1(i, carry):
            phase1(i)
            return carry
        lax.fori_loop(0, 2, l1, 0)
        c_xa1.wait()

        def l2(i, carry):
            phase1(i, _spread(weave(relayout(i - 2), transpose_wo(i - 2)), SPN, 3 * NP))
            return carry
        lax.fori_loop(2, S // T1, l2, 0)

        c_woa.wait()
        c_mem.wait()
        c_xb0.wait()
        mem[...] = mem0[...].astype(F32)
        xbs[...] = xbt[:, 0:TB].astype(F32).T
        wps = []
        for p in range(NP):
            if p % 2 == 0:
                last = _spread(transpose_wo(NPIECE + p // 2), 2, 2)
            wk_ = min(W, D - 128 * p)
            wp = _dot(sel_q[p][1][:, :wk_], woa[128 * p:128 * p + wk_, :])
            for f, z in zip(last[p % 2], _pace(wp, len(last[p % 2]))):
                f(z)
            wps.append(wp.astype(BF16))
        wop[...] = _u32(jnp.concatenate(wps, axis=0).astype(F32).T.astype(BF16))
        r = _iota((RG + 8, 2 * RG), 0)
        c = _iota((RG + 8, 2 * RG), 1)
        head = jnp.where(r < RG, (r >= DA).astype(I32) + (r >= 2 * DA).astype(I32) + (r >= 3 * DA).astype(I32),
                         r & 3)
        keep = head == (c & 3)
        r = _iota((RG + 8, RG + 8), 0)
        c = _iota((RG + 8, RG + 8), 1)
        perm = jnp.where(c == jnp.where(r < RG, (r & 3) * DA + (r >> 2), r), 1.0, 0.0).astype(BF16)
        for g in range(NG):
            kv = _dot(perm, jnp.where(keep, kvacc[g], 0.0).astype(BF16)).astype(BF16)
            kvl[g] = _u32(kv)
            nums[g] = _dot(kv, _b16(phq[g, :, 0:TB]))

    @pl.when(step == 1)
    def _late():
        cols(xbt_hbm, xbt, 2 * TB, S, SEM_XB1).wait()

    st2 = {}
    nxt0 = pl.multiple_of(jnp.minimum(step + 1, NSTEP - 1) * TB, TB)
    ro = D // NO

    def a_num_next():
        for g in range(NG):
            nums[g] = _dot(_b16(kvl[g]), _b16(phq[g, :, pl.ds(nxt0, TB)]))

    def a_norm():
        os_ = []
        for g in range(NG):
            r = nums[g]
            den = r[RG:RG + 8, :] + 1e-6
            os_.append((r[:RG, :].reshape(DA // 2, 8, TB) * (1.0 / den)[None]).reshape(RG, TB))
        st2["ot"] = jnp.concatenate(os_, axis=0).astype(BF16)

    def a_out(p):
        st2["out", p] = _dot(_b16(wop[p * ro // 2:(p + 1) * ro // 2, :]), st2["ot"])
        if p == NO - 1:
            outa = jnp.concatenate([st2.pop(("out", k)) for k in range(NO)], axis=0).T
            o_ref[:, 0:D] = outa.astype(BF16)

    def b_x_next():
        xbs[...] = xbt[:, pl.ds(nxt0, TB)].astype(F32).T

    end = HB + LAG_OUT - 1
    fills = [{2: a_norm, end: functools.partial(a_out, 0)},
             {end: functools.partial(a_out, 1)},
             {4: b_x_next, end: functools.partial(a_out, 2)},
             {end: a_num_next}]

    cexp = scale * LOG2E

    def b_step(hmat, first, fill):
        bias = biasa[...] if first else biasb[...]
        ok = bias == 0.0
        acc = None
        qkv, pv, oo = {}, {}, {}

        def proj(h):
            q, k, v = [_dot(hmat, _b16(wr[h * 3 + i])).astype(BF16) for i in range(3)]
            if first:
                sq[h] = _u32(q[32:48])
                sk[h] = _u32(k)
                sv[h] = _u32(v)
                q = q[0:32]
            else:
                q = jnp.concatenate([q, _b16(sq[h])], axis=0)
                k = jnp.concatenate([_b16(sk[h]), k], axis=0)
                v = jnp.concatenate([_b16(sv[h]), v], axis=0)
            qkv[h] = (q, k, v)

        def score(h):
            q, k, v = qkv.pop(h)
            s = jnp.where(ok, _dot_nt(q, k), bias)
            m = jnp.max(s, axis=-1, keepdims=True)
            p = jnp.exp2((s - m) * cexp)
            pv[h] = (p.astype(BF16), jnp.sum(p, axis=-1, keepdims=True), v)

        def mix(h):
            p, l, v = pv.pop(h)
            oo[h] = (_dot(p, v) * _recip(l)).astype(BF16)

        def outp(h, acc):
            o = oo.pop(h)
            parts = [_dot(o, _b16(wob[j, h * 64:(h + 1) * 64, :])) for j in range(5)]
            return parts if acc is None else [a + b for a, b in zip(acc, parts)]

        for t in range(end + 1):
            if t < HB:
                proj(t)
            if 0 <= t - LAG_SCORE < HB:
                score(t - LAG_SCORE)
            if 0 <= t - LAG_MIX < HB:
                mix(t - LAG_MIX)
            if t < HB:
                hs = [t - OUT_RATE * LAG_OUT] if t >= OUT_RATE * LAG_OUT else []
            else:
                h1 = HB - OUT_RATE * (end - t)
                hs = range(h1 - OUT_RATE, h1)
            for h in hs:
                acc = outp(h, acc)
            if t in fill:
                fill[t]()
        acc[4] = acc[4][:, 0:64]
        return jnp.concatenate(acc, axis=1)

    m_cur = mem[...]
    xs = [xbs[p * 64:(p + 1) * 64, :] for p in range(TB // 64)]
    for p in range(TB // 64):
        x = xs[p]
        ra = b_step(jnp.concatenate([m_cur, x[0:40]], axis=0).astype(BF16), True, fills[2 * p])
        rb = b_step(jnp.concatenate([ra[0:8], x[40:64]], axis=0).astype(BF16), False, fills[2 * p + 1])
        m_cur = rb[0:8]
        ob = jnp.concatenate([ra[8:32], rb[32:48], rb[8:32]], axis=0)
        o_ref[p * 64:(p + 1) * 64, D:2 * D] = ob.astype(BF16)
    mem[...] = m_cur


@functools.partial(jax.jit, static_argnames=("B_seg_len",))
def pallas_concat_heads__linear_kernel_hedgehog__memory_aug_recurrent_mem_tr__prompt_kernel(A_x, A_wqkv, A_w_phi, A_wo, B_x, B_mem0, B_Wq, B_Wk, B_Wv, B_Wo, B_seg_len):
    assert B_seg_len == SEG
    assert A_x.shape == (1, S, D) and B_x.shape == (1, S, D) and B_Wq.shape == (D, HB, DB)
    hbm = pl.BlockSpec(memory_space=pltpu.HBM)
    out = pl.pallas_call(
        _kernel,
        grid=(NSTEP,),
        in_specs=[hbm] * 10,
        out_specs=pl.BlockSpec((TB, 2 * D), lambda i: (i, 0)),
        out_shape=jax.ShapeDtypeStruct((S, 2 * D), BF16),
        scratch_shapes=[
            pltpu.VMEM((D, S), BF16),
            pltpu.VMEM((D, 3 * D), BF16),
            pltpu.VMEM((D, D), BF16),
            pltpu.VMEM((3 * D * HB, DB), BF16),
            pltpu.VMEM((2, 8 * 33, 128), U32),
            pltpu.VMEM((3 * HB, D // 2, DB), U32),
            pltpu.VMEM((HB, D, DB), BF16),
            pltpu.VMEM((5, HB * DB // 2, 128), U32),
            pltpu.VMEM((3, D // 2, D), U32),
            pltpu.VMEM((D // 2, D), U32),
            pltpu.VMEM((NG, RG + 8, 2 * RG), F32),
            pltpu.VMEM((NG, (RG + 8) // 2, 2 * RG), U32),
            pltpu.VMEM((NG, RG, S), U32),
            pltpu.VMEM((MEM, D), F32),
            pltpu.VMEM((HB, 8, DB), U32),
            pltpu.VMEM((HB, 24, DB), U32),
            pltpu.VMEM((HB, 24, DB), U32),
            pltpu.VMEM((32, 48), F32),
            pltpu.VMEM((48, 80), F32),
            pltpu.VMEM((TB, D), F32),
            pltpu.VMEM((DA, DA, HA), BF16),
            pltpu.VMEM((MEM, D), BF16),
            pltpu.VMEM((D, S), BF16),
            pltpu.VMEM((NG, RG + 8, TB), F32),
            pltpu.SemaphoreType.DMA((NSEM,)),
        ],
        compiler_params=pltpu.CompilerParams(
            dimension_semantics=("arbitrary",),
            vmem_limit_bytes=100 * 1024 * 1024,
        ),
        name="hedgehog_memtr",
    )(
        A_x.reshape(S, D).T, A_wqkv, jnp.transpose(A_w_phi, (1, 2, 0)), A_wo,
        B_x.reshape(S, D).T, B_mem0.reshape(MEM, D),
        B_Wq.reshape(D * HB, DB), B_Wk.reshape(D * HB, DB), B_Wv.reshape(D * HB, DB),
        jnp.transpose(B_Wo, (0, 2, 1)),
    )
    return out.reshape(1, S, 2 * D)
```

```python
import functools

import jax
import jax.numpy as jnp
from jax import lax
import jax.experimental.pallas as pl
import jax.experimental.pallas.tpu as pltpu

F32 = jnp.float32
BF16 = jnp.bfloat16
U32 = jnp.uint32
I32 = jnp.int32
NT = (((1,), (1,)), ((), ()))
LOG2E = 1.4426950408889634

S = 2048
D = 576
HA = 32
DA = 18
NP = 4
HP = 72
RG = 72
NS = 16
RS = 40
HB = 32
DB = 128
MEM = 8
SEG = 32
TB = 128
NSTEP = S // TB
T1 = 256
CH = 18
NPIECE = 3 * (D // 16) // CH
PROWS = CH * 16 * HB
HW = 4
NWO = HB // HW
PACE = 4
LAT = ((450, 0, 400, 700, 400, 400, 16, 45),
       (250, 600, 300, 800, 350, 350, 14, 60),
       (450, 0, 300, 700, 250, 400, 16, 60),
       (200, 500, 450, 650, 350, 350, 13, 60))
PRIO = "MGCSTRV"
NO = 3
(SEM_WK, SEM_WV, SEM_WQ, SEM_WOA, SEM_XA0, SEM_XA1, SEM_PHI, SEM_MEM, SEM_XB0, SEM_XB1, SEM_WO) = range(11)
SEM_RAW = SEM_WO + NWO
SEM_OUT = SEM_RAW + NPIECE
NSEM = SEM_OUT + NSTEP + 1
PADR = 32


def _iota(shape, dim):
    return lax.broadcasted_iota(I32, shape, dim)


def _recip(x):
    r = pl.reciprocal(x, approx=True)
    return r * (2.0 - x * r)


def _b16(v):
    return pltpu.bitcast(v, BF16)


def _u32(v):
    return pltpu.bitcast(v, U32)


def _dot(a, b):
    return jnp.dot(a, b, preferred_element_type=F32)


def _dot_nt(a, b):
    return lax.dot_general(a, b, NT, preferred_element_type=F32)


def _feature_map(p):
    t = p.shape[-1]
    x = p.reshape(9, 8, t)
    low = _iota((8, t), 0) < 4

    def fold(r, op):
        r = op(r, pltpu.roll(r, 4, 0))
        return op(r, pltpu.roll(r, 2, 0))

    def soft(red, op, fill, arg):
        m0 = fold(op(red(x[0:4], axis=0), jnp.where(low, x[4], fill)), op)
        m1 = fold(op(red(x[5:9], axis=0), jnp.where(low, fill, x[4])), op)
        e4 = jnp.exp2(arg(x[4], jnp.where(low, m0, m1)))
        e0 = jnp.concatenate([jnp.exp2(arg(x[0:4], m0[None])), jnp.where(low, e4, 0.0)[None]], axis=0)
        e1 = jnp.concatenate([jnp.where(low, 0.0, e4)[None], jnp.exp2(arg(x[5:9], m1[None]))], axis=0)
        return [e * _recip(fold(jnp.sum(e, axis=0), jnp.add))[None] for e in (e0, e1)]
    pos = soft(jnp.max, jnp.maximum, -jnp.inf, lambda v, m: v - m)
    neg = soft(jnp.min, jnp.minimum, jnp.inf, lambda v, m: m - v)
    return [jnp.concatenate([pos[k], neg[k]], axis=0).reshape(2 * RS, t).astype(BF16) for k in range(2)]


def _pace(res, n):
    pos = [(r, c) for c in range(res.shape[1] // 128) for r in range(res.shape[0] // 8)]
    pos = [pos[(2 * i + 1) * len(pos) // (2 * n)] for i in range(n)]
    return [(_u32(res[8 * r:8 * r + 8, 128 * c:128 * c + 128]) >> 16) >> 16 for r, c in pos]


def _spread(fs, n):
    return [fs[len(fs) * k // n:len(fs) * (k + 1) // n] for k in range(n)]


def _schedule(idx):
    lat, (keep, ts) = LAT[idx][:6], LAT[idx][6:]
    n = HB // 2
    rows, rwo = (48, 32) if idx % 2 == 0 else (32, 48)
    ready, mix_after = {}, {}
    nxt = {c: 0 for c in "TSCGMROV"}
    order = []
    t = 0.0
    np_ = 0
    while nxt["O"] < n:
        cand = [c for c in PRIO if ready.get((c, nxt[c]), 1e18) <= t]
        if nxt["R"] == n - 1 and "R" in cand and nxt["O"] < n - 1:
            cand.remove("R")
        o_ok = ready.get(("O", nxt["O"]), 1e18) <= t
        if cand:
            c = cand[0]
        elif np_ < HB:
            c = "O" if (o_ok and np_ % 2 == 0 and nxt["O"] < np_ // 2 - keep) else "P"
        elif o_ok and not (nxt["O"] == n - 1 and nxt["R"] < n):
            c = "O"
        else:
            t = min(v for (c, i), v in ready.items() if nxt[c] == i and v > t)
            continue
        if c == "P":
            i = np_
            np_ += 1
        else:
            i = nxt[c]
            nxt[c] += 1
        lp, lt, ls, lc, lg, lm = [v * ts / 100 for v in lat] if np_ == HB else lat
        order.append((c, i))
        if c == "S":
            ready["V", i] = t
        t += dict(P=9 * rows, T=0, S=2 * rows, C=rows, V=8 * rows, G=rows, M=2 * rows,
                  R=144 if idx == 3 else 16, O=8 * rwo)[c] / 4
        if c == "P" and i % 2 == 1:
            ready["T", i // 2] = t + lp
        elif c == "T":
            ready["S", i] = t + lt
        elif c == "S":
            ready["C", i] = t + ls
        elif c == "C":
            ready["G", i] = t + lc
        elif c in "VG":
            mix_after.setdefault(i, []).append(t + (lp if c == "V" else lg))
            if len(mix_after[i]) == 2:
                ready["M", i] = max(mix_after[i])
        elif c == "M":
            ready["R", i] = ready["O", i] = t + lm
    return order


def _kernel(xat_hbm, wqkv_hbm, wphi_hbm, woa_hbm, xbt_hbm, mem0_hbm, wq_hbm, wk_hbm, wv_hbm, wobt_hbm,
            o_ref,
            xat, wqkv, woa, raw, stage, wr, wobt, wob, wobp, wt, wop, kvacc, kvl, phq,
            mem, qf, kf, vf, kx, vx, k2, v2, o2, hx, h2, biasa, biasb, xbs, wphi, mem0, xbt, nums, ox, of,
            biasz, obuf, wkt, sems):
    step = pl.program_id(0)
    scale = DB ** (-0.5)

    def cols(src, dst, a, b, sem):
        return pltpu.make_async_copy(src.at[:, pl.ds(a, b - a)], dst.at[:, pl.ds(a, b - a)], sems.at[sem])

    @pl.when(step == 0)
    def _prologue():
        c_phi = pltpu.make_async_copy(wphi_hbm, wphi, sems.at[SEM_PHI])
        c_wk = cols(wqkv_hbm, wqkv, 512, 1152, SEM_WK)
        c_wv = cols(wqkv_hbm, wqkv, 1152, 1728, SEM_WV)
        c_wq = cols(wqkv_hbm, wqkv, 0, 512, SEM_WQ)
        c_xa0 = cols(xat_hbm, xat, 0, 2 * T1, SEM_XA0)
        c_xa1 = cols(xat_hbm, xat, 2 * T1, S, SEM_XA1)
        c_woa = pltpu.make_async_copy(woa_hbm, woa, sems.at[SEM_WOA])
        c_mem = pltpu.make_async_copy(mem0_hbm, mem0, sems.at[SEM_MEM])
        c_xb0 = cols(xbt_hbm, xbt, 0, 2 * TB, SEM_XB0)
        for c in (c_phi, c_wk, c_wq, c_wv, c_xa0, c_xa1):
            c.start()
        for p in range(NWO):
            if p < NPIECE:
                src = (wq_hbm, wk_hbm, wv_hbm)[p // 2]
                pltpu.make_async_copy(src.at[pl.ds((p % 2) * PROWS, PROWS)], raw.at[pl.ds(p * PROWS, PROWS)],
                                      sems.at[SEM_RAW + p]).start()
            if p == NPIECE:
                for c in (c_woa, c_mem, c_xb0):
                    c.start()
            pltpu.make_async_copy(wobt_hbm.at[pl.ds(p * HW, HW)], wobt.at[pl.ds(p * HW, HW)],
                                  sems.at[SEM_WO + p]).start()
        cols(xbt_hbm, xbt, 2 * TB, S, SEM_XB1).start()

        neg = -1e9 / scale
        r = _iota((48, 128), 0)
        c = _iota((48, 128), 1) & 63
        own = ((r < 40) & (c < 40)) | ((r >= 40) & (c >= 48))
        vis = (r < 8) | ((r < 40) & (r >= c)) | ((r >= 40) & (c - 16 <= r))
        biasa[...] = jnp.where(own & vis, 0.0, jnp.where(own, neg, -jnp.inf)).astype(F32)
        r = _iota((32, 128), 0)
        c = _iota((32, 128), 1) & 63
        own = (c < 32) | ((c >= 40) & (c < 48))
        vis = (r < 8) | (c >= 40) | (r >= c)
        biasb[...] = jnp.where(own & vis, 0.0, jnp.where(own, neg, -jnp.inf)).astype(F32)
        r = _iota((8, 128), 0)
        c = _iota((8, 128), 1) & 63
        own = (c < 32) | ((c >= 40) & (c < 48))
        vis = (c < 8) | ((c >= 40) & (c - 40 <= r))
        biasz[...] = jnp.where(own & vis, 0.0, jnp.where(own, neg, -jnp.inf)).astype(F32)
        for ref in (qf, kx, vx, hx):
            ref[...] = jnp.zeros(ref.shape, ref.dtype)
        kvacc[...] = jnp.zeros(kvacc.shape, F32)

        W = 256
        WF = 640

        def split(off, shape):
            cc = _iota(shape, 1) - off
            hh = jnp.floor((cc.astype(F32) + 0.5) * (1.0 / DA)).astype(I32)
            return hh, cc - hh * DA

        rr = _iota((D, WF), 0)
        hh, dd = split(0, (8, WF))
        src = jnp.where(hh < HA, dd * HA + hh, -1)[0:1, :]
        hot = jnp.where(rr == src, 1.0, 0.0).astype(BF16)
        c_phi.wait()
        wcat = jnp.concatenate([wphi[d].astype(F32) for d in range(DA)], axis=1).astype(BF16)
        t1 = _dot(wcat, hot).astype(BF16)

        def row_ids(shape):
            rho = _iota(shape, 0)
            pair = (rho >= 36).astype(I32) + (rho >= 72).astype(I32) + (rho >= 108).astype(I32)
            j = rho - 36 * pair
            return 2 * pair + (j & 1), j >> 1
        _, f_r = row_ids((2 * RG, DA))
        full = _dot(jnp.where(f_r == _iota((2 * RG, DA), 1), 1.0, 0.0).astype(BF16), t1)
        fulls = [full, pltpu.roll(full, 64, 1)]
        h_r, f_r = row_ids((2 * RG, W))

        def selectors(p, k):
            h_c, d_c = split(16 * p + 64 * k, (8, W))
            hm = h_r == h_c[0:1, :]
            bd = jnp.where(hm, fulls[k][:, 128 * p:128 * p + W], 0.0)
            pm = jnp.where(hm & (f_r == d_c[0:1, :]), 1.0, 0.0)
            return bd.astype(BF16), pm.astype(BF16)

        sel_k = [selectors(p, 1)[0] for p in range(NP)]
        c_wk.wait()
        sel_q = [selectors(p, 0) for p in range(NP)]
        for p in range(NP):
            wt[1, p * HP:(p + 1) * HP, :] = _u32(
                (_dot_nt(sel_k[p], wqkv[:, 512 + 128 * p:512 + 128 * p + W]) * LOG2E).astype(BF16))
        c_wq.wait()
        for p in range(NP):
            if p == 2:
                c_wv.wait()
                for j in range(5):
                    n = 128 if j < 4 else 64
                    blk = wqkv[:, 1152 + 128 * j:1152 + 128 * j + n].astype(F32)
                    wt[2, 64 * j:64 * j + n // 2, :] = _u32(blk.T.astype(BF16))
            wt[0, p * HP:(p + 1) * HP, :] = _u32(
                (_dot_nt(sel_q[p][0], wqkv[:, 128 * p:128 * p + W]) * LOG2E).astype(BF16))

        def phase1(i, extra=()):
            t0 = pl.multiple_of(i * T1, T1)
            xv = xat.at[:, pl.ds(t0, T1)]
            ones = jnp.ones((8, T1), F32)
            vts, phis = {}, {}

            def proj(m, t, k):
                res = _dot(_b16(wt[m, t * HP:(t + 1) * HP, :]), xv[...])
                if extra:
                    for f, z in zip(extra[k], _pace(res, len(extra[k]))):
                        f(z)
                return res
            for t in range(NP + 2):
                if t < NP:
                    pq = proj(0, t, 3 * t)
                    for g2 in range(2):
                        for k, phi in enumerate(_feature_map(pq[g2 * RG:(g2 + 1) * RG])):
                            phq[4 * t + 2 * g2 + k, :, pl.ds(t0, T1)] = _u32(phi)
                    pk = proj(1, t, 3 * t + 1)
                    vt = proj(2, t, 3 * t + 2)
                    for g2 in range(2):
                        for k, phi in enumerate(_feature_map(pk[g2 * RG:(g2 + 1) * RG])):
                            r0 = g2 * RG + k * 32
                            vts[4 * t + 2 * g2 + k] = jnp.concatenate([vt[r0:r0 + RS], ones], axis=0).astype(BF16)
                            phis[4 * t + 2 * g2 + k] = phi
                if t >= 2:
                    for g in range(4 * t - 8, 4 * t - 4):
                        kvacc[g] += _dot_nt(vts.pop(g), phis.pop(g))

        def relayout(p):
            rawp = raw.at[pl.ds(pl.multiple_of(p * PROWS, PROWS), PROWS)]
            pltpu.make_async_copy(rawp, rawp, sems.at[SEM_RAW + p]).wait()
            m = p // 2
            d0 = (p - m * 2) * (CH * 8)

            def put(c, q0, z):
                st = stage.at[c % 2]
                for q in range(q0, q0 + 8 // PACE):
                    u = _u32(rawp[c * 512 + q * 64:c * 512 + (q + 1) * 64, :])
                    st[pl.ds(q * 33, 32), :] = u | jnp.concatenate([z] * 4, axis=0)

            def get(c, j0, z):
                st = stage.at[c % 2]
                rr = pl.multiple_of(d0 + c * 8, 8)
                for j in range(j0, j0 + 16 // PACE):
                    e = st[pl.ds(j, 8, stride=33), :] | z
                    o = st[pl.ds(16 + j, 8, stride=33), :]
                    wr[(2 * j) * 3 + m, pl.ds(rr, 8), :] = (e & U32(0xffff)) | (o << 16)
                    wr[(2 * j + 1) * 3 + m, pl.ds(rr, 8), :] = (e >> 16) | (o & U32(0xffff0000))
            fs = []
            for c in range(CH):
                fs += [functools.partial(put, c, k * 8 // PACE) for k in range(PACE)]
                fs += [functools.partial(get, c, k * 16 // PACE) for k in range(PACE)]
            return fs

        def transpose_wo(p):
            src = wobt.at[pl.ds(p * HW, HW)]
            pltpu.make_async_copy(src, src, sems.at[SEM_WO + p]).wait()
            dst = wob.at[:, pl.ds(pl.multiple_of(p * HW * 64, 64), HW * 64), :]
            dstp = wobp.at[pl.ds(p * (HW // 2), HW // 2)]

            def flip(u, z):
                u = jnp.concatenate([u[0:8] | z, u[8:]], axis=0)
                return _u32(_b16(u).astype(F32).T.astype(BF16))

            def block(hh, j, z):
                dst[j, hh * 64:(hh + 1) * 64, :] = flip(_u32(src[hh, j * 128:(j + 1) * 128, :]), z)

            def pair(i, z):
                dstp[i] = flip(jnp.concatenate([_u32(src[2 * i + 1, 512:576, :]), _u32(src[2 * i, 512:576, :])],
                                               axis=0), z)
            return ([functools.partial(block, hh, j) for hh in range(HW) for j in range(4)]
                    + [functools.partial(pair, i) for i in range(HW // 2)])

        def weave(a, b):
            n = len(a) * 4 // 5
            out = []
            for k in range(len(b)):
                out += [b[k]] + a[n * k // len(b):n * (k + 1) // len(b)]
            return out + a[n:]

        def l1(i, carry):
            phase1(i)
            return carry
        c_xa0.wait()
        lax.fori_loop(0, 2, l1, 0)
        c_xa1.wait()

        def l2(i, carry):
            phase1(i, _spread(weave(relayout(i - 2), transpose_wo(i - 2)), 3 * NP))
            return carry
        lax.fori_loop(2, S // T1, l2, 0)

        c_woa.wait()
        c_mem.wait()
        c_xb0.wait()

        def key_tail(i, z):
            u = jnp.concatenate([wr[(2 * i + 1) * 3 + 1, 256:288, :], wr[2 * i * 3 + 1, 256:288, :]], axis=0)
            u = jnp.concatenate([u[0:8] | z, u[8:]], axis=0)
            wkt[i] = _u32(_b16(u).astype(F32).T.astype(BF16))
        last = _spread(transpose_wo(NPIECE) + transpose_wo(NPIECE + 1)
                       + [functools.partial(key_tail, i) for i in range(HB // 2)], NP)
        mem[...] = mem0[...].astype(F32)
        xbs[...] = xbt[:, 0:TB].astype(F32).T
        wps = []
        for p in range(NP):
            wk_ = min(W, D - 128 * p)
            wp = _dot(sel_q[p][1][:, :wk_], woa[128 * p:128 * p + wk_, :])
            for f, z in zip(last[p], _pace(wp, len(last[p]))):
                f(z)
            wps.append(wp.astype(BF16))
        wop[...] = _u32(jnp.concatenate(wps, axis=0).astype(F32).T.astype(BF16))
        for k in range(2):
            r = _iota((RS + 8, 2 * RS), 0)
            c = _iota((RS + 8, 2 * RS), 1)
            keep = jnp.where(r < RS, (r >= 4 * k + DA).astype(I32), r & 1) == (c & 1)
            r = _iota((RS + 8, RS + 8), 0)
            c = _iota((RS + 8, RS + 8), 1)
            j = r - 4 * k
            src = jnp.where(r >= RS, r, jnp.where((j >= 0) & (j < 36), 4 * k + (j & 1) * DA + (j >> 1), -1))
            perm = jnp.where(c == src, 1.0, 0.0).astype(BF16)
            for g in range(k, NS, 2):
                kv = _dot(perm, jnp.where(keep, kvacc[g], 0.0).astype(BF16)).astype(BF16)
                kvl[g] = _u32(kv)
                nums[g] = _dot(kv, _b16(phq[g, :, 0:TB]))

    def out_copy(row, n, sem):
        return pltpu.make_async_copy(obuf.at[pl.ds(PADR + row, n)], o_ref.at[pl.ds(row, n)], sems.at[SEM_OUT + sem])

    @pl.when(step == 1)
    def _late():
        cols(xbt_hbm, xbt, 2 * TB, S, SEM_XB1).wait()
        out_copy(0, TB - 32, 0).start()

    @pl.when(step > 1)
    def _flush():
        out_copy(pl.multiple_of((step - 1) * TB - 32, 32), TB, step - 1).start()

    st2 = {}
    blk = obuf.at[pl.ds(pl.multiple_of(step * TB, TB), PADR + TB)]

    nxt0 = pl.multiple_of(jnp.minimum(step + 1, NSTEP - 1) * TB, TB)
    ro = D // NO

    def a_num_next():
        for g in range(NS):
            nums[g] = _dot(_b16(kvl[g]), _b16(phq[g, :, pl.ds(nxt0, TB)]))

    def a_norm():
        os_ = []
        for g in range(NS):
            r = nums[g]
            den = r[RS:RS + 8, :] + 1e-6
            o = (r[:RS, :].reshape(5, 8, TB) * (1.0 / den)[None]).reshape(RS, TB)
            if g % 2 == 0:
                os_ += [o[0:32], o[32:40]]
            else:
                os_[-1] = os_[-1] + o[0:8]
                os_.append(o[8:40])
        st2["ot"] = jnp.concatenate(os_, axis=0).astype(BF16)

    def a_out(p):
        st2["out", p] = _dot(_b16(wop[p * ro // 2:(p + 1) * ro // 2, :]), st2["ot"])
        if p == NO - 1:
            outa = jnp.concatenate([st2.pop(("out", k)) for k in range(NO)], axis=0).T
            blk[PADR:PADR + TB, 0:D] = outa.astype(BF16)

    def b_x_next():
        xbs[...] = xbt[:, pl.ds(nxt0, TB)].astype(F32).T

    end = "end"
    fills = [{10: a_norm, end: functools.partial(a_out, 0)},
             {end: functools.partial(a_out, 1)},
             {end: functools.partial(a_out, 2)},
             {15: b_x_next, end: a_num_next}]

    cexp = scale * LOG2E
    final = step == NSTEP - 1

    def b_step(hrows, idx, fill):
        first = idx % 2 == 0
        nq = 48 if first else 32
        hmat = hrows.astype(BF16)
        bias = biasa[...] if first else biasb[...]
        if idx == 3:
            bias = jnp.concatenate([jnp.where(final, biasz[...], bias[0:8]), bias[8:32]], axis=0)
        ok = bias == 0.0
        left = _iota((nq, 128), 1) < 64
        hr = hmat[:, 512:576].astype(F32)
        if first:
            hk = jnp.concatenate([hr, hx[...]], axis=0)
            h2[...] = hr[32:48]
        else:
            prev = h2[...]
            hk = jnp.concatenate([hr, prev, jnp.zeros((16, 64), F32)], axis=0)
            hx[...] = jnp.concatenate([hr[0:8], prev[8:16]], axis=0)
        z64 = jnp.zeros((64, 64), F32)
        anti = jnp.concatenate([jnp.concatenate([z64, hk], axis=1), jnp.concatenate([hk, z64], axis=1)], axis=0)
        rg = anti.astype(BF16)
        rc = anti.T.astype(BF16)
        pad16 = jnp.zeros((16, DB), BF16)
        qkv, sc, pp, gg, oo, om, st = {}, {}, {}, {}, {}, {}, {}

        def add(key, val):
            st[key] = val if key not in st else st[key] + val

        def keys(h, i, f32s, x_tile, tile2):
            r = _dot(hmat[:, :512], _b16(wr[h * 3 + i, 0:256, :]))
            rb = r.astype(BF16)
            if first:
                f32s[h] = r[40:48]
                tile2[h] = _u32(rb[32:48])
                return jnp.concatenate([rb, _b16(x_tile[h])], axis=0)
            x_tile[h] = _u32(jnp.concatenate([r[0:8], f32s[h]], axis=0).astype(BF16))
            return jnp.concatenate([rb, _b16(tile2[h])] + ([pad16] if i == 1 or h % 2 == 0 else []), axis=0)

        def proj(h):
            k = keys(h, 1, kf, kx, k2)
            q = _dot(hmat, _b16(wr[h * 3]))
            if first:
                qb = jnp.concatenate([q[0:40], qf[h]], axis=0).astype(BF16)
                qf[h] = q[40:48]
            else:
                if idx == 3:
                    q = jnp.concatenate([jnp.where(final, qf[h], q[0:8]), q[8:32]], axis=0)
                qb = q.astype(BF16)
            qkv[h] = (qb, k)

        def values(i):
            for h in (2 * i, 2 * i + 1):
                qkv["v", h] = keys(h, 2, vf, vx, v2)

        def both(a, b, h):
            return jnp.concatenate([a, b] if h % 2 == 0 else [b, a], axis=0)

        def tstep(i):
            if not first:
                kt = jnp.concatenate([qkv[2 * i][1], qkv[2 * i + 1][1]], axis=0)
                kt = _u32(kt.astype(F32).T.astype(BF16))
                wtile = wkt[i]
                l64 = _iota((64, 128), 1) < 64
                sc["t", i] = (_b16(jnp.where(l64, kt, wtile)), _b16(jnp.where(l64, wtile, kt)))

        def score(i):
            tiles = sc.pop(("t", i), None)
            for h in (2 * i, 2 * i + 1):
                q, k = qkv.pop(h)
                if tiles is None:
                    sc[h] = _dot_nt(q, both(k, _b16(wr[h * 3 + 1, 256:288, :]), h))
                else:
                    sc[h] = _dot(q, tiles[h % 2])

        def corr(i):
            s0, s1 = sc.pop(2 * i), sc.pop(2 * i + 1)
            s = jnp.where(left, s0, s1) + _dot(jnp.where(left, s1, s0).astype(BF16), rc)
            s = jnp.where(ok, s, bias)
            m0 = jnp.max(jnp.where(left, s, -jnp.inf), axis=-1, keepdims=True)
            m1 = jnp.max(jnp.where(left, -jnp.inf, s), axis=-1, keepdims=True)
            p = jnp.exp2((s - jnp.where(left, m0, m1)) * cexp)
            l0 = jnp.sum(jnp.where(left, p, 0.0), axis=-1, keepdims=True)
            l1 = jnp.sum(jnp.where(left, 0.0, p), axis=-1, keepdims=True)
            pp[i] = (p, l0, l1)

        def gstep(i):
            gg[i] = _dot(pp[i][0].astype(BF16), rg)

        def mix(i):
            p, l0, l1 = pp.pop(i)
            g = gg.pop(i)
            for h, l, lhs in ((2 * i, l0, jnp.where(left, p, g)), (2 * i + 1, l1, jnp.where(left, g, p))):
                v = qkv.pop(("v", h))
                o = _dot(lhs.astype(BF16)[:, :64 + v.shape[0]],
                         both(v, _b16(wr[h * 3 + 2, 256:288, :]), h)) * _recip(l)
                ob = o.astype(BF16)
                om[h] = o[0:8]
                if first:
                    oo[h] = ob[0:32]
                    o2[h] = _u32(ob[32:48])
                    ox[h, (idx // 2) * 32:(idx // 2) * 32 + 16, :] = _u32(o[8:40].astype(BF16))
                    of[h] = o[40:48]
                else:
                    oo[h] = jnp.concatenate([ob, _b16(o2[h])], axis=0)
                    xt = jnp.concatenate([o[8:32], of[h]], axis=0).astype(BF16)
                    if idx == 1:
                        ox[h, 16:32, :] = _u32(xt)
                    else:
                        om["x", h] = xt

        def rem(i):
            r = _dot(jnp.concatenate([om.pop(2 * i + 1), om.pop(2 * i)], axis=0).astype(BF16), _b16(wobp[i]))
            if i == HB // 2 - 1:
                add("l", pltpu.roll(st.pop("r"), 64, 1))
                add("l", r[0:8] + pltpu.roll(r[8:16], 64, 1))
            else:
                add("l", r[0:8])
                add("r", r[8:16])
            if idx == 3:
                for h in (2 * i, 2 * i + 1):
                    xr = jnp.concatenate([_b16(ox[h]), om.pop(("x", h))], axis=0)
                    add("x", _dot_nt(wobt[h, 512:576, :], xr))

        def outp(h):
            o = oo.pop(h)
            for j in range(4):
                add(j, _dot(o, _b16(wob[j, h * 64:(h + 1) * 64, :])))

        stage = dict(T=tstep, S=score, C=corr, G=gstep, M=mix, R=rem, P=proj, V=values)
        for c, i in _schedule(idx):
            if c == "O":
                outp(2 * i)
                outp(2 * i + 1)
            else:
                stage[c](i)
            if c == "P" and i in fill:
                fill[i]()
        fill[end]()
        res = jnp.concatenate([st[j] for j in range(4)], axis=1)
        return res, jnp.concatenate([res[0:8], st["l"][:, 0:64]], axis=1), st.get("x")

    m_cur = mem[...]
    xs = [xbs[p * 64:(p + 1) * 64, :] for p in range(TB // 64)]
    for p in range(TB // 64):
        x = xs[p]
        ra, m_cur, _ = b_step(jnp.concatenate([m_cur, x[0:40]], axis=0), 2 * p, fills[2 * p])
        rb, m_cur, xr = b_step(jnp.concatenate([m_cur, x[40:64]], axis=0), 2 * p + 1, fills[2 * p + 1])
        r0 = PADR + p * 64
        blk[r0:r0 + 24, D:D + 512] = ra[8:32].astype(BF16)
        blk[r0 + 40:r0 + 64, D:D + 512] = rb[8:32].astype(BF16)
        blk[r0 + 24:r0 + 32, D:D + 512] = rb[32:40].astype(BF16)
        blk[r0 - 32:r0 - 24, D:D + 512] = rb[40:48].astype(BF16)
    mem[...] = m_cur
    xr = jnp.concatenate([jnp.zeros((64, TB), F32), xr], axis=0).T[:, 64:128].astype(BF16)
    for p in range(TB // 64):
        r0 = PADR + p * 64
        blk[r0:r0 + 32, D + 512:2 * D] = xr[64 * p:64 * p + 32]
        blk[r0 + 40:r0 + 64, D + 512:2 * D] = xr[64 * p + 32:64 * p + 56]
        blk[r0 - 32:r0 - 24, D + 512:2 * D] = xr[64 * p + 56:64 * p + 64]

    @pl.when(final)
    def _finish():
        tail = [out_copy(S - 160, 64, NSTEP - 1), out_copy(S - 96, 96, NSTEP)]
        tail[0].start()
        obuf[PADR + S - 32:PADR + S - 24, D:2 * D] = m_cur.astype(BF16)
        tail[1].start()
        out_copy(0, TB - 32, 0).wait()
        for i in range(1, NSTEP - 1):
            out_copy(i * TB - 32, TB, i).wait()
        for c in tail:
            c.wait()


@jax.jit
def pallas_concat_heads__linear_kernel_hedgehog__memory_aug_recurrent_mem_tr__prompt_kernel(
        A_x, A_wqkv, A_w_phi, A_wo, B_x, B_mem0, B_Wq, B_Wk, B_Wv, B_Wo, B_seg_len):
    del B_seg_len
    assert A_x.shape == (1, S, D) and B_x.shape == (1, S, D) and B_Wq.shape == (D, HB, DB)
    hbm = pl.BlockSpec(memory_space=pltpu.MemorySpace.HBM)
    out = pl.pallas_call(
        _kernel,
        grid=(NSTEP,),
        in_specs=[hbm] * 10,
        out_specs=hbm,
        out_shape=jax.ShapeDtypeStruct((S, 2 * D), BF16),
        scratch_shapes=[
            pltpu.VMEM((D, S), BF16),
            pltpu.VMEM((D, 3 * D), BF16),
            pltpu.VMEM((D, D), BF16),
            pltpu.VMEM((3 * D * HB, DB), BF16),
            pltpu.VMEM((2, 8 * 33, 128), U32),
            pltpu.VMEM((3 * HB, D // 2, DB), U32),
            pltpu.VMEM((HB, D, DB), BF16),
            pltpu.VMEM((4, HB * DB // 2, 128), U32),
            pltpu.VMEM((HB // 2, DB // 2, 128), U32),
            pltpu.VMEM((3, D // 2, D), U32),
            pltpu.VMEM((D // 2, D), U32),
            pltpu.VMEM((NS, RS + 8, 2 * RS), F32),
            pltpu.VMEM((NS, (RS + 8) // 2, 2 * RS), U32),
            pltpu.VMEM((NS, RS, S), U32),
            pltpu.VMEM((MEM, D), F32),
            pltpu.VMEM((HB, 8, DB), F32),
            pltpu.VMEM((HB, 8, DB), F32),
            pltpu.VMEM((HB, 8, DB), F32),
            pltpu.VMEM((HB, 8, DB), U32),
            pltpu.VMEM((HB, 8, DB), U32),
            pltpu.VMEM((HB, 8, DB), U32),
            pltpu.VMEM((HB, 8, DB), U32),
            pltpu.VMEM((HB, 8, DB), U32),
            pltpu.VMEM((16, 64), F32),
            pltpu.VMEM((16, 64), F32),
            pltpu.VMEM((48, 128), F32),
            pltpu.VMEM((32, 128), F32),
            pltpu.VMEM((TB, D), F32),
            pltpu.VMEM((DA, DA, HA), BF16),
            pltpu.VMEM((MEM, D), BF16),
            pltpu.VMEM((D, S), BF16),
            pltpu.VMEM((NS, RS + 8, TB), F32),
            pltpu.VMEM((HB, 48, DB), U32),
            pltpu.VMEM((HB, 8, DB), F32),
            pltpu.VMEM((8, 128), F32),
            pltpu.VMEM((PADR + S, 2 * D), BF16),
            pltpu.VMEM((HB // 2, 64, 128), U32),
            pltpu.SemaphoreType.DMA((NSEM,)),
        ],
        compiler_params=pltpu.CompilerParams(
            dimension_semantics=("arbitrary",),
            vmem_limit_bytes=100 * 1024 * 1024,
        ),
        name="hedgehog_memtr",
    )(
        A_x.reshape(S, D).T, A_wqkv, jnp.transpose(A_w_phi, (1, 2, 0)), A_wo,
        B_x.reshape(S, D).T, B_mem0.reshape(MEM, D),
        B_Wq.reshape(D * HB, DB), B_Wk.reshape(D * HB, DB), B_Wv.reshape(D * HB, DB),
        jnp.transpose(B_Wo, (0, 2, 1)),
    )
    return out.reshape(1, S, 2 * D)
```
